```python
import os as _os
_os.environ.setdefault('JAX_PLATFORMS', 'cpu')
import jax
import jax.numpy as jnp

def _softmax(x, axis=-1):
    return jax.nn.softmax(x, axis=axis)

def _gelu(x):
    return jax.nn.gelu(x, approximate=True)

def _silu(x):
    return jax.nn.silu(x)

def _sigmoid(x):
    return jax.nn.sigmoid(x)

def _layernorm(x, axis=-1, eps=1e-05):
    m = jnp.mean(x, axis=axis, keepdims=True)
    v = jnp.var(x, axis=axis, keepdims=True)
    return (x - m) / jnp.sqrt(v + eps)

def _scatter_add(tgt, idx, src, axis=0):
    return tgt.at[idx].add(src)

def _segment_sum(src, seg, n):
    return jax.ops.segment_sum(src, seg, n)

class _Rng:

    def __init__(self, key):
        self._k = key

    def _next(self):
        self._k, sub = jax.random.split(self._k)
        return sub

    def normal(self, shape):
        return jax.random.normal(self._next(), shape, dtype=jnp.bfloat16)

    def randint(self, lo, hi, shape):
        return jax.random.randint(self._next(), shape, lo, hi, dtype=jnp.int32)

    def uniform(self, shape, lo=0.0, hi=1.0):
        return jax.random.uniform(self._next(), shape, jnp.bfloat16, lo, hi)

    def permutation(self, n):
        return jax.random.permutation(self._next(), n)
kernel_name = 'sequential_preLN__linear_attn_block__mixer_gmlp__prompt'

def setup_inputs():
    _rng = _Rng(jax.random.key(int.from_bytes(__import__("os").urandom(4), "little")))
    _w = lambda a: (lambda t: t.astype(jnp.bfloat16) if jnp.issubdtype(t.dtype, jnp.floating) else t)(jnp.asarray(a))

    def _A_setup():
        B, S, D = (1, 2048, 512)
        return {'x': _w((lambda *s: _rng.normal(s) * 0.05)(B, S, D)), 'wqkv': _w((lambda *s: _rng.normal(s) * 0.05)(D, 3 * D)), 'wo': _w((lambda *s: _rng.normal(s) * 0.05)(D, D))}
    _A_in = _A_setup()

    def _B_setup():
        B, S, D, F = (1, 2048, 512, 1792)
        Fh = F // 2
        return {'x': _w((lambda *s: _rng.normal(s) * 0.05)(B, S, D)), 'w_in': _w((lambda *s: _rng.normal(s) * 0.4)(D, 2 * Fh)), 'w_sp': _w(0.01 * (lambda *s: _rng.normal(s) * 0.4)(S, S)), 'b_sp': _w(1.0 + 0.01 * (lambda *s: _rng.normal(s) * 0.05)(S)), 'w_out': _w((lambda *s: _rng.normal(s) * 0.05)(Fh, D))}
    _B_in = _B_setup()
    return {'A_x': _A_in['x'], 'A_wqkv': _A_in['wqkv'], 'A_wo': _A_in['wo'], 'B_x': _B_in['x'], 'B_w_in': _B_in['w_in'], 'B_w_sp': _B_in['w_sp'], 'B_b_sp': _B_in['b_sp'], 'B_w_out': _B_in['w_out']}

def reference(A_x, A_wqkv, A_wo, B_x, B_w_in, B_w_sp, B_b_sp, B_w_out):

    def _A_ref(x, wqkv, wo):
        B, S, D = x.shape
        H = 32
        Dh = D // H
        qkv = (lambda x, *d: x.transpose(*d))((x @ wqkv).reshape(B, S, 3, H, Dh), 2, 0, 3, 1, 4)
        q, k, v = (qkv[0], qkv[1], qkv[2])
        phi = lambda t: jnp.where(t > 0, t + 1, jnp.exp(t)) + 1e-06
        pq, pk = (phi(q), phi(k))
        kv = jnp.einsum('bhsd,bhse->bhde', pk, v)
        z = jnp.einsum('bhsd->bhd', pk)
        num = jnp.einsum('bhqd,bhde->bhqe', pq, kv)
        den = jnp.einsum('bhqd,bhd->bhq', pq, z)[..., None] + 1e-06
        o = num / den
        return (lambda x, *d: x.transpose(*d))(o, 0, 2, 1, 3).reshape(B, S, D) @ wo

    def _B_ref(x, w_in, w_sp, b_sp, w_out):
        B, S, D = x.shape
        F = w_in.shape[-1]
        Fh = F // 2
        z = _gelu(jnp.einsum('bsd,df->bsf', x, w_in))
        z1 = z[..., :Fh].copy()
        z2 = _layernorm(z[..., Fh:], axis=-1)
        g = jnp.einsum('ts,bsf->btf', w_sp, z2) + b_sp[None, :, None]
        return jnp.einsum('bsf,fd->bsd', z1 * g, w_out)
    x = A_x
    h = x + _A_ref(_layernorm(x, axis=-1), A_wqkv, A_wo)
    h2 = h + _B_ref(_layernorm(h, axis=-1), B_w_in, B_w_sp, B_b_sp, B_w_out)
    return h2
```

```python
import numpy as np
import jax
import jax.numpy as jnp
from jax import lax
import jax.experimental.pallas as pl
import jax.experimental.pallas.tpu as pltpu

S, D, H, FH = 2048, 512, 32, 896
DH = D // H
TM = 256
NT = S // TM
NL = D // 128
BF = jnp.bfloat16
F32 = jnp.float32
C1 = float(np.sqrt(2.0 / np.pi))
C2 = float(np.sqrt(2.0 / np.pi) * 0.044715)


def _ln(x):
    n = x.shape[-1]
    m = jnp.sum(x, axis=-1, keepdims=True) * (1.0 / n)
    d = x - m
    v = jnp.sum(d * d, axis=-1, keepdims=True) * (1.0 / n)
    return d * lax.rsqrt(v + 1e-5)


def _phi(t):
    return jnp.where(t > 0, t + 1.0, jnp.exp(t)) + 1e-6


def _gelu(x):
    u = x * (C1 + C2 * (x * x))
    hx = 0.5 * x
    return hx * jnp.tanh(u) + hx


def _recip(d):
    r = pl.reciprocal(d, approx=True)
    return r * (2.0 - d * r)


def _dot(a, b):
    return jnp.dot(a, b, preferred_element_type=F32)


def _kernel(x_hbm, wqkv_hbm, wo_hbm, win_hbm, wsp_hbm, bsp_hbm, wout_hbm, out_hbm,
            x_s, wqkv_s, wo_s, win_s, wsp_s, bsp_s, wout_s,
            pq_s, m_s, zbt_s, h_s, z1_s, z2_s, o_s, xn_s, kv_s, z_s, b32_s,
            sem_in, sem_o):
    def rows(i):
        if isinstance(i, int):
            return pl.ds(i * TM, TM)
        return pl.ds(pl.multiple_of(i * TM, TM), TM)

    cp_x01 = pltpu.make_async_copy(x_hbm.at[pl.ds(0, 2 * TM)], x_s.at[pl.ds(0, 2 * TM)], sem_in.at[0])
    cp_xr = pltpu.make_async_copy(x_hbm.at[pl.ds(2 * TM, S - 2 * TM)], x_s.at[pl.ds(2 * TM, S - 2 * TM)], sem_in.at[1])
    cp_wqkv = pltpu.make_async_copy(wqkv_hbm, wqkv_s, sem_in.at[2])
    cp_wo = pltpu.make_async_copy(wo_hbm, wo_s, sem_in.at[3])
    cp_win = pltpu.make_async_copy(win_hbm, win_s, sem_in.at[4])
    cp_bsp = pltpu.make_async_copy(bsp_hbm, bsp_s, sem_in.at[5])
    cp_wout = pltpu.make_async_copy(wout_hbm, wout_s, sem_in.at[6])
    cp_wsp = pltpu.make_async_copy(wsp_hbm, wsp_s, sem_in.at[7])

    def cp_o(i):
        return pltpu.make_async_copy(o_s.at[rows(i)], out_hbm.at[rows(i)], sem_o.at[i])

    def ln_x(i):
        return _ln(x_s[rows(i), :].astype(F32)).astype(BF)

    cp_x01.start()
    cp_wqkv.start()
    cp_x01.wait()
    cp_xr.start()
    xn_s[rows(0), :] = ln_x(0)
    kv_s[...] = jnp.zeros(kv_s.shape, F32)
    z_s[...] = jnp.zeros(z_s.shape, F32)
    cp_wqkv.wait()
    cp_wo.start()
    cp_win.start()
    cp_bsp.start()

    def a1(i, c):
        @pl.when(i == 1)
        def _():
            cp_xr.wait()
        xn = xn_s[rows(i), :]
        nx = jnp.minimum(i + 1, NT - 1)
        xn_s[rows(nx), :] = ln_x(nx)
        k = _dot(xn, wqkv_s[:, D:2 * D])
        v = _dot(xn, wqkv_s[:, 2 * D:3 * D]).astype(BF)
        pk = _phi(k)
        z_s[...] += jnp.sum(pk.reshape(TM // 8, 8, D), axis=0)
        pkT = [pk[:, j * 128:(j + 1) * 128].T.astype(BF) for j in range(NL)]
        pq_s[rows(i), :] = _phi(_dot(xn, wqkv_s[:, 0:D])).astype(BF)
        for j in range(NL):
            kv_s[j] += _dot(pkT[j], v[:, j * 128:(j + 1) * 128])
        return c

    lax.fori_loop(0, NT, a1, 0)

    row = lax.broadcasted_iota(jnp.int32, (128, 128), 0) // DH
    col = lax.broadcasted_iota(jnp.int32, (128, 128), 1) // DH
    same = row == col
    zall = jnp.sum(z_s[...], axis=0, keepdims=True)
    for j in range(NL):
        zrow = zall[:, j * 128:(j + 1) * 128]
        zbt_s[j] = jnp.where(same, jnp.broadcast_to(zrow, (128, 128)), 0.0).astype(BF)

    cp_wo.wait()
    cp_win.wait()
    cp_wout.start()
    cp_wsp.start()

    def st_den(i):
        return [lax.dot_general(pq_s[rows(i), j * 128:(j + 1) * 128], zbt_s[j],
                                (((1,), (1,)), ((), ())), preferred_element_type=F32) for j in range(NL)]

    def st_h(i, den):
        h = x_s[rows(i), :].astype(F32)
        for j in range(NL):
            pq = pq_s[rows(i), j * 128:(j + 1) * 128]
            pqs = (pq.astype(F32) * _recip(den[j] + 1e-6)).astype(BF)
            h = h + _dot(pqs, m_s[j * 128:(j + 1) * 128, :])
        h_s[rows(i), :] = h
        xn_s[rows(i), :] = _ln(h).astype(BF)

    def st_z2(i, z2):
        z2_s[rows(i), :] = _ln(_gelu(z2)).astype(BF)

    den = st_den(0)
    for j in range(NL):
        kvb = jnp.where(same, kv_s[j], 0.0).astype(BF)
        m_s[j * 128:(j + 1) * 128, :] = _dot(kvb, wo_s[j * 128:(j + 1) * 128, :]).astype(BF)
    st_h(0, den)

    def st_z1(i, hn, lo, hi):
        z1_s[rows(i), lo:hi] = _dot(hn, win_s[:, lo:hi]).astype(BF)

    def st_pqs(i, den):
        return [(pq_s[rows(i), j * 128:(j + 1) * 128].astype(F32) * _recip(den[j] + 1e-6)).astype(BF)
                for j in range(NL)]

    def st_m(i, pqs):
        h = x_s[rows(i), :].astype(F32)
        for j in range(NL):
            h = h + _dot(pqs[j], m_s[j * 128:(j + 1) * 128, :])
        h_s[rows(i), :] = h
        return h

    def st_lnh(i, h):
        xn_s[rows(i), :] = _ln(h).astype(BF)

    def a2(i, c):
        hn = xn_s[rows(i), :]
        den = st_den(i + 1)
        st_z2(i, _dot(hn, win_s[:, FH:2 * FH]))
        st_z1(i, hn, 0, 512)
        h = st_m(i + 1, st_pqs(i + 1, den))
        st_lnh(i + 1, h)
        st_z1(i, hn, 512, FH)
        return c

    lax.fori_loop(0, NT - 1, a2, 0)
    hn = xn_s[rows(NT - 1), :]
    z2 = _dot(hn, win_s[:, FH:2 * FH])
    st_z2(NT - 1, z2)
    z1_s[rows(NT - 1), :] = _dot(hn, win_s[:, 0:FH]).astype(BF)

    cp_bsp.wait()
    cp_wout.wait()
    cp_wsp.wait()
    b32_s[...] = bsp_s[...].astype(F32)

    def b(i, c):
        g = _dot(wsp_s[rows(i), :], z2_s[...])
        bcol = jnp.concatenate(
            [jnp.broadcast_to(b32_s[pl.ds(i * (TM // 128) + t, 1), :], (128, 128)).T
             for t in range(TM // 128)], axis=0)
        bfull = jnp.concatenate([bcol] * (FH // 128), axis=1)
        gz = (_gelu(z1_s[rows(i), :].astype(F32)) * (g + bfull)).astype(BF)
        y = _dot(gz, wout_s[...])
        o_s[rows(i), :] = (h_s[rows(i), :] + y).astype(BF)
        pltpu.make_async_copy(o_s.at[rows(i)], out_hbm.at[rows(i)], sem_o.at[i]).start()
        return c

    lax.fori_loop(0, NT, b, 0)
    for i in range(NT):
        cp_o(i).wait()


@jax.jit
def pallas_sequential_preLN__linear_attn_block__mixer_gmlp__prompt_kernel(
    A_x, A_wqkv, A_wo, B_x, B_w_in, B_w_sp, B_b_sp, B_w_out
):
    del B_x
    x2 = A_x.reshape(S, D)
    b2 = B_b_sp.reshape(S // 128, 128)
    anyspec = pl.BlockSpec(memory_space=pl.ANY)
    out = pl.pallas_call(
        _kernel,
        out_shape=jax.ShapeDtypeStruct((S, D), BF),
        in_specs=[anyspec] * 7,
        out_specs=anyspec,
        scratch_shapes=[
            pltpu.VMEM((S, D), BF), pltpu.VMEM((D, 3 * D), BF), pltpu.VMEM((D, D), BF),
            pltpu.VMEM((D, 2 * FH), BF), pltpu.VMEM((S, S), BF), pltpu.VMEM((S // 128, 128), BF),
            pltpu.VMEM((FH, D), BF),
            pltpu.VMEM((S, D), BF),
            pltpu.VMEM((D, D), BF),
            pltpu.VMEM((NL, 128, 128), BF),
            pltpu.VMEM((S, D), F32),
            pltpu.VMEM((S, FH), BF),
            pltpu.VMEM((S, FH), BF),
            pltpu.VMEM((S, D), BF),
            pltpu.VMEM((S, D), BF),
            pltpu.VMEM((NL, 128, 128), F32),
            pltpu.VMEM((8, D), F32),
            pltpu.VMEM((S // 128, 128), F32),
            pltpu.SemaphoreType.DMA((8,)), pltpu.SemaphoreType.DMA((NT,)),
        ],
        compiler_params=pltpu.CompilerParams(vmem_limit_bytes=100 * 1024 * 1024),
    )(x2, A_wqkv, A_wo, B_w_in, B_w_sp, b2, B_w_out)
    return out.reshape(1, S, D)
```

```python
import numpy as np
import jax
import jax.numpy as jnp
from jax import lax
import jax.experimental.pallas as pl
import jax.experimental.pallas.tpu as pltpu

S, D, HEADS, FH = 2048, 512, 32, 896
DH = D // HEADS
TM = 256
NT = S // TM
NL = D // 128
RC = 32
NO = 2
BF = jnp.bfloat16
F32 = jnp.float32
C1 = float(np.sqrt(2.0 / np.pi))
C2 = float(np.sqrt(2.0 / np.pi) * 0.044715)


def _ln(x, eps=1e-5):
    n = x.shape[-1]
    m = jnp.sum(x, axis=-1, keepdims=True) * (1.0 / n)
    d = x - m
    v = jnp.sum(d * d, axis=-1, keepdims=True) * (1.0 / n)
    return d * lax.rsqrt(v + eps)


def _phi(t):
    return jnp.where(t > 0, t + 1.0, jnp.exp(t)) + 1e-6


def _gelu(x):
    hx = 0.5 * x
    return hx * jnp.tanh(x * (C1 + C2 * (x * x))) + hx


def _gelu_x2(x):
    return x * (1.0 + jnp.tanh(x * (C1 + C2 * (x * x))))


def _recip(d):
    r = pl.reciprocal(d, approx=True)
    return r * (2.0 - d * r)


def _dot(a, b):
    return jnp.dot(a, b, preferred_element_type=F32)


def _loop(lo, hi, body, u):
    n = (hi - lo) // u
    if n > 0:
        def grp(g, c):
            for t in range(u):
                body(lo + g * u + t)
            return c
        lax.fori_loop(0, n, grp, 0)
    for i in range(lo + n * u, hi):
        body(i)


def _kernel(x_hbm, wqkv_hbm, wo_hbm, win_hbm, wsp_hbm, bsp_hbm, wout_hbm, out_hbm,
            x_s, wqkv_s, wo_s, win_s, wsp_s, bsp_s, wout_s,
            pq_s, m_s, zbt_s, h_s, z1_s, z2_s, o_s, xn_s, g_s, z_s, b32_s,
            sem_w, sem_x, sem_o):
    def sub(i, r, n):
        if isinstance(i, int):
            return pl.ds(i * TM + r, n)
        return pl.ds(pl.multiple_of(i * TM + r, n), n)

    def rows(i):
        return sub(i, 0, TM)

    def cp_x(i):
        return pltpu.make_async_copy(x_hbm.at[rows(i)], x_s.at[rows(i)], sem_x.at[i])

    def cp_o(i, t):
        cs = pl.ds(t * (D // NO), D // NO)
        return pltpu.make_async_copy(o_s.at[rows(i), cs], out_hbm.at[rows(i), cs], sem_o.at[i, t])

    def cp(src, dst, k):
        return pltpu.make_async_copy(src, dst, sem_w.at[k])

    cp_wq, cp_wk, cp_wv = [
        cp(wqkv_hbm.at[:, pl.ds(t * D, D)], wqkv_s.at[:, pl.ds(t * D, D)], t) for t in range(3)]
    cp_wo = cp(wo_hbm, wo_s, 3)
    cp_win = cp(win_hbm, win_s, 4)
    cp_bsp = cp(bsp_hbm, bsp_s, 5)
    cp_wout = cp(wout_hbm, wout_s, 6)
    cp_wsp = cp(wsp_hbm, wsp_s, 7)


    def ln_x(i):
        xn_s[rows(i), :] = _ln(x_s[rows(i), :].astype(F32)).astype(BF)

    def st_k(xn):
        return _dot(xn, wqkv_s[:, D:2 * D])

    def st_q(i, xn, lo, hi):
        pq_s[rows(i), lo:hi] = _phi(_dot(xn, wqkv_s[:, lo:hi])).astype(BF)

    def st_pk(k, first=False):
        pk = _phi(k)
        zs = jnp.sum(pk.reshape(TM // 8, 8, D), axis=0)
        z_s[...] = zs if first else z_s[...] + zs
        return [pk[:, j * 128:(j + 1) * 128].T.astype(BF) for j in range(NL)]

    def st_g(pkT, xn, first=False):
        for j in range(NL):
            c = _dot(pkT[j], xn)
            g_s[j] = c if first else g_s[j] + c

    cp_x(0).start()
    cp_wk.start()
    cp_x(0).wait()
    cp_wq.start()
    cp_x(1).start()
    ln_x(0)
    cp_wk.wait()
    xn = xn_s[rows(0), :]
    k = st_k(xn)
    cp_wq.wait()
    cp_x(1).wait()
    cp_x(2).start()
    cp_x(3).start()
    ln_x(1)
    pkT = st_pk(k, True)
    st_q(0, xn, 0, D)
    st_g(pkT, xn, True)

    def a1(i, c):
        cp_x(i + 1).wait()

        @pl.when(i == 1)
        def _():
            for t in range(4, NT):
                cp_x(t).start()

        @pl.when(i == 2)
        def _():
            cp_wv.start()
            cp_wo.start()
            cp_win.start()
            cp_bsp.start()
        xn = xn_s[rows(i), :]
        ln_x(i + 1)
        pkT = st_pk(st_k(xn))
        st_q(i, xn, 0, 256)
        st_g(pkT, xn)
        st_q(i, xn, 256, D)
        return c

    lax.fori_loop(1, NT - 1, a1, 0)

    cp_wv.wait()
    cp_wo.wait()
    cp_win.wait()
    cp_wout.start()
    cp_wsp.start()
    xn7 = xn_s[rows(NT - 1), :]
    pkT = st_pk(st_k(xn7))
    st_q(NT - 1, xn7, 0, 128)
    st_g(pkT, xn7)

    same = (lax.broadcasted_iota(jnp.int32, (128, 128), 0) // DH
            == lax.broadcasted_iota(jnp.int32, (128, 128), 1) // DH)
    zall = jnp.sum(z_s[...], axis=0, keepdims=True)
    for j in range(NL):
        zrow = zall[:, j * 128:(j + 1) * 128]
        zbt_s[j] = jnp.where(same, jnp.broadcast_to(zrow, (128, 128)), 0.0).astype(BF)

    kvs = []
    for j in range(NL):
        g = g_s[j]
        ghi = g.astype(BF)
        glo = (g - ghi.astype(F32)).astype(BF)
        wv = wqkv_s[:, 2 * D + j * 128:2 * D + (j + 1) * 128]
        kvs.append(_dot(ghi, wv) + _dot(glo, wv))
    st_q(NT - 1, xn7, 128, 256)
    for j in range(NL):
        kvb = jnp.where(same, kvs[j], 0.0).astype(BF)
        m_s[j * 128:(j + 1) * 128, :] = _dot(kvb, wo_s[j * 128:(j + 1) * 128, :]).astype(BF)

    def st_den(i):
        return [lax.dot_general(pq_s[rows(i), j * 128:(j + 1) * 128], zbt_s[j],
                                (((1,), (1,)), ((), ())), preferred_element_type=F32) for j in range(NL)]

    def st_h(i, den):
        pqs = [(pq_s[rows(i), j * 128:(j + 1) * 128].astype(F32) * _recip(den[j] + 1e-6)).astype(BF)
               for j in range(NL)]
        h = x_s[rows(i), :].astype(F32)
        for j in range(NL):
            h = h + _dot(pqs[j], m_s[j * 128:(j + 1) * 128, :])
        h_s[rows(i), :] = h
        for r in range(0, TM, RC):
            xn_s[sub(i, r, RC), :] = _ln(h[r:r + RC]).astype(BF)

    def st_z2(i, hn):
        z2 = _dot(hn, win_s[:, FH:2 * FH])
        for r in range(0, TM, RC):
            z2_s[sub(i, r, RC), :] = _ln(_gelu_x2(z2[r:r + RC]), 4e-5).astype(BF)

    def st_z1(i, hn, lo, hi):
        z1_s[rows(i), lo:hi] = _dot(hn, win_s[:, lo:hi]).astype(BF)

    den = st_den(0)
    st_q(NT - 1, xn7, 256, 384)
    st_h(0, den)
    st_q(NT - 1, xn7, 384, D)

    def a2(i):
        hn = xn_s[rows(i), :]
        den = st_den(i + 1)
        st_z2(i, hn)
        st_z1(i, hn, 0, 512)
        st_h(i + 1, den)
        st_z1(i, hn, 512, FH)

    _loop(0, NT - 1, a2, 2)
    hn = xn_s[rows(NT - 1), :]
    st_z2(NT - 1, hn)
    st_z1(NT - 1, hn, 0, FH)

    cp_bsp.wait()
    cp_wout.wait()
    cp_wsp.wait()
    b32_s[...] = bsp_s[...].astype(F32)

    def b(i):
        g = _dot(wsp_s[rows(i), :], z2_s[...])
        bcol = jnp.concatenate(
            [jnp.broadcast_to(b32_s[pl.ds(i * (TM // 128) + t, 1), :], (128, 128)).T
             for t in range(TM // 128)], axis=0)
        bfull = jnp.concatenate([bcol] * (FH // 128), axis=1)
        gz = (_gelu(z1_s[rows(i), :].astype(F32)) * (g + bfull)).astype(BF)
        for t in range(NO):
            cs = slice(t * (D // NO), (t + 1) * (D // NO))
            o_s[rows(i), cs] = (h_s[rows(i), cs] + _dot(gz, wout_s[:, cs])).astype(BF)
            cp_o(i, t).start()

    _loop(0, NT, b, 4)
    for i in range(NT):
        for t in range(NO):
            cp_o(i, t).wait()


@jax.jit
def pallas_sequential_preLN__linear_attn_block__mixer_gmlp__prompt_kernel(
    A_x, A_wqkv, A_wo, B_x, B_w_in, B_w_sp, B_b_sp, B_w_out
):
    del B_x
    anyspec = pl.BlockSpec(memory_space=pl.ANY)
    out = pl.pallas_call(
        _kernel,
        out_shape=jax.ShapeDtypeStruct((S, D), BF),
        in_specs=[anyspec] * 7,
        out_specs=anyspec,
        scratch_shapes=[
            pltpu.VMEM((S, D), BF),
            pltpu.VMEM((D, 3 * D), BF),
            pltpu.VMEM((D, D), BF),
            pltpu.VMEM((D, 2 * FH), BF),
            pltpu.VMEM((S, S), BF),
            pltpu.VMEM((S // 128, 128), BF),
            pltpu.VMEM((FH, D), BF),
            pltpu.VMEM((S, D), BF),
            pltpu.VMEM((D, D), BF),
            pltpu.VMEM((NL, 128, 128), BF),
            pltpu.VMEM((S, D), F32),
            pltpu.VMEM((S, FH), BF),
            pltpu.VMEM((S, FH), BF),
            pltpu.VMEM((S, D), BF),
            pltpu.VMEM((S, D), BF),
            pltpu.VMEM((NL, 128, D), F32),
            pltpu.VMEM((8, D), F32),
            pltpu.VMEM((S // 128, 128), F32),
            pltpu.SemaphoreType.DMA((8,)),
            pltpu.SemaphoreType.DMA((NT,)),
            pltpu.SemaphoreType.DMA((NT, NO)),
        ],
        compiler_params=pltpu.CompilerParams(vmem_limit_bytes=100 * 1024 * 1024),
    )(A_x.reshape(S, D), A_wqkv, A_wo, B_w_in, B_w_sp, B_b_sp.reshape(S // 128, 128), B_w_out)
    return out.reshape(1, S, D)
```
